```python
import jax
import jax.numpy as jnp

def _softmax(x, axis=-1):
    return jax.nn.softmax(x, axis=axis)
def _gelu(x):
    return jax.nn.gelu(x, approximate=True)
def _silu(x):
    return jax.nn.silu(x)
def _sigmoid(x):
    return jax.nn.sigmoid(x)
def _layernorm(x, axis=-1, eps=1e-5):
    m = jnp.mean(x, axis=axis, keepdims=True)
    v = jnp.var(x, axis=axis, keepdims=True)
    return (x - m) / jnp.sqrt(v + eps)
def _scatter_add(tgt, idx, src, axis=0):
    return tgt.at[idx].add(src)
def _segment_sum(src, seg, n):
    return jax.ops.segment_sum(src, seg, n)
class _Rng:
    def __init__(self, key):
        self._k = key
    def _next(self):
        self._k, sub = jax.random.split(self._k)
        return sub
    def normal(self, shape):
        return jax.random.normal(self._next(), shape, dtype=jnp.bfloat16)
    def randint(self, lo, hi, shape):
        return jax.random.randint(self._next(), shape, lo, hi, dtype=jnp.int32)
    def uniform(self, shape, lo=0.0, hi=1.0):
        return jax.random.uniform(self._next(), shape, jnp.bfloat16, lo, hi)
    def permutation(self, n):
        return jax.random.permutation(self._next(), n)


kernel_name = 'standalone__detection_seg_fpn_lateral__vision'

def setup_inputs():
    _rng = _Rng(jax.random.key(int.from_bytes(__import__("os").urandom(4), "little")))
    _w = (lambda a: (lambda t: t.astype(jnp.bfloat16) if jnp.issubdtype(t.dtype, jnp.floating) else t)(jnp.asarray(a)))
    H = W = (384 // 2) * 2
    C = 384
    k = 1
    return {
        "c_fine": _w((lambda *s: _rng.normal(s) * 0.05)(1, H, W, C)),
        "p_coarse": _w((lambda *s: _rng.normal(s) * 0.05)(1, H // 2, W // 2, C)),
        "w_lat": _w((lambda *s: _rng.normal(s) * 0.05)(C, C)),
        "w_out": _w((lambda *s: _rng.normal(s) * 0.05)(k, k, C, C)),
    }

def reference(c_fine, p_coarse, w_lat, w_out):
    B, H, W, C = c_fine.shape
    k = 1
    lat = jnp.einsum("bhwc,cd->bhwd", c_fine, w_lat)
    up = jnp.repeat(jnp.repeat(p_coarse, 2, axis=1), 2, axis=2)
    m = lat + up
    pad = k // 2
    mp = jnp.pad(m, ((0, 0), (pad, pad), (pad, pad), (0, 0)))
    o = None
    for di in range(k):
        for dj in range(k):
            t = jnp.einsum("bhwc,cd->bhwd", mp[:, di:di + H, dj:dj + W, :], w_out[di, dj])
            o = t if o is None else o + t
    return o
```

```python
import jax
import jax.numpy as jnp
import jax.experimental.pallas as pl
import jax.experimental.pallas.tpu as pltpu

BH = 16
NP = 14
KT = 14
S = 1024
TW = 32
INIT = 64
PER = 8
TAIL = 2


@jax.jit
def pallas_standalone__detection_seg_fpn_lateral__vision_kernel(
    c_fine: jax.Array,
    p_coarse: jax.Array,
    w_lat: jax.Array,
    w_out: jax.Array,
):
    B, H, W, C = c_fine.shape
    assert B == 1 and w_out.shape == (1, 1, C, C)
    nblk = H // BH
    pb = BH // 2
    last = nblk - 1
    th = BH * W // S
    nwin = S // TW
    na = H * W // S
    npair2 = (nblk - KT) * pb
    rest0 = INIT + PER * npair2
    assert H % BH == 0 and (BH * W) % S == 0 and S % TW == 0
    assert nblk - NP <= KT and NP < nblk and INIT <= KT * nwin
    assert rest0 <= nblk * nwin
    for m in range(npair2):
        assert (INIT + PER * (m + 1) - 1) // nwin < KT + m // pb

    def kernel(c_hbm, p_hbm, wl_hbm, wo_hbm, o_hbm,
               buf, pbuf, wl_v, wo_v, wf_v, csem, psem, wsem, osem, tsem):
        buf_w = buf.reshape(na, S, C)

        def c_rd(j):
            rows = pl.ds(j * BH, BH)
            return pltpu.make_async_copy(c_hbm.at[rows], buf.at[rows], csem.at[j])

        def p_rd(j, slot):
            return pltpu.make_async_copy(
                p_hbm.at[pl.ds(j * pb, pb)], pbuf.at[slot], psem.at[j])

        def p_last_main():
            return pltpu.make_async_copy(
                p_hbm.at[pl.ds(last * pb, pb - TAIL)],
                pbuf.at[last % NP, pl.ds(0, pb - TAIL)], psem.at[last])

        def p_last_tail():
            return pltpu.make_async_copy(
                p_hbm.at[pl.ds(last * pb + pb - TAIL, TAIL)],
                pbuf.at[last % NP, pl.ds(pb - TAIL, TAIL)], tsem.at[0])

        def o_wr(t):
            b = t // nwin
            w0 = (t % nwin) * TW
            if not isinstance(t, int):
                w0 = pl.multiple_of(w0, TW)
            win = (pl.ds(b * th, th), pl.ds(w0, TW))
            return pltpu.make_async_copy(buf_w.at[win], o_hbm.at[win], osem.at[b])

        wl_cp = pltpu.make_async_copy(wl_hbm, wl_v, wsem.at[0])
        wo_cp = pltpu.make_async_copy(wo_hbm, wo_v, wsem.at[1])
        wl_cp.start()
        wo_cp.start()

        def issue(j, carry):
            p_rd(j, j).start()
            c_rd(j).start()
            return carry

        jax.lax.fori_loop(0, NP, issue, 0)
        for j in range(NP, nblk):
            c_rd(j).start()

        wl_cp.wait()
        wo_cp.wait()
        wf_v[...] = jnp.dot(
            wl_v[...], wo_v[...], preferred_element_type=jnp.float32
        ).astype(jnp.bfloat16)

        def row_pair(j, slot, h):
            q = jnp.dot(pbuf[slot, h], wo_v[...], preferred_element_type=jnp.float32)
            u = pltpu.bitcast(q.astype(jnp.bfloat16).astype(jnp.float32), jnp.uint32)
            up = pltpu.bitcast(u | (u >> 16), jnp.bfloat16).astype(jnp.float32)
            for r in range(2):
                row = j * BH + 2 * h + r
                acc = jnp.dot(buf[row], wf_v[...], preferred_element_type=jnp.float32)
                buf[row] = (acc + up).astype(jnp.bfloat16)

        def block1(j, carry):
            slot = j % NP
            p_rd(j, slot).wait()
            c_rd(j).wait()

            def body(h, c2):
                row_pair(j, slot, h)
                return c2

            jax.lax.fori_loop(0, pb, body, 0)

            @pl.when(j + NP < last)
            def _():
                p_rd(j + NP, slot).start()

            @pl.when(j + NP == last)
            def _():
                p_last_main().start()
                p_last_tail().start()

            return carry

        jax.lax.fori_loop(0, KT, block1, 0)

        for j in range(KT, nblk):
            c_rd(j).wait()
        for j in range(KT, last):
            p_rd(j, j % NP).wait()
        p_last_main().wait()
        for t in range(INIT):
            o_wr(t).start()
        p_last_tail().wait()

        def body2(m, carry):
            for k in range(PER):
                o_wr(INIT + PER * m + k).start()
            j = KT + m // pb
            row_pair(j, j % NP, m % pb)
            return carry

        jax.lax.fori_loop(0, npair2, body2, 0)
        for t in range(rest0, nblk * nwin):
            o_wr(t).start()
        for b in range(nblk):
            rows = pl.ds(b * th, th)
            pltpu.make_async_copy(buf_w.at[rows], o_hbm.at[rows], osem.at[b]).wait()

    bf16 = jnp.bfloat16
    out = pl.pallas_call(
        kernel,
        in_specs=[pl.BlockSpec(memory_space=pl.ANY)] * 4,
        out_specs=pl.BlockSpec(memory_space=pl.ANY),
        out_shape=jax.ShapeDtypeStruct((na, S, C), c_fine.dtype),
        scratch_shapes=[
            pltpu.VMEM((H, W, C), bf16),
            pltpu.VMEM((NP, pb, W // 2, C), bf16),
            pltpu.VMEM((C, C), bf16),
            pltpu.VMEM((C, C), bf16),
            pltpu.VMEM((C, C), bf16),
            pltpu.SemaphoreType.DMA((nblk,)),
            pltpu.SemaphoreType.DMA((nblk,)),
            pltpu.SemaphoreType.DMA((2,)),
            pltpu.SemaphoreType.DMA((nblk,)),
            pltpu.SemaphoreType.DMA((1,)),
        ],
        compiler_params=pltpu.CompilerParams(vmem_limit_bytes=127 * 1024 * 1024),
    )(
        c_fine.reshape(H, W, C),
        p_coarse.reshape(H // 2, W // 2, C),
        w_lat,
        w_out.reshape(C, C),
    )
    return out.reshape(B, H, W, C)
```

```python
import jax
import jax.numpy as jnp
import jax.experimental.pallas as pl
import jax.experimental.pallas.tpu as pltpu

M1 = 113
D = 2
NRING = 4
MT = 64
LAG = 2
S = 2048
TH = 6
TW = 16
INIT = 64
PER = 16
TAIL = 128


@jax.jit
def pallas_standalone__detection_seg_fpn_lateral__vision_kernel(
    c_fine: jax.Array,
    p_coarse: jax.Array,
    w_lat: jax.Array,
    w_out: jax.Array,
):
    B, H, W, C = c_fine.shape
    assert B == 1 and w_out.shape == (1, 1, C, C)
    assert p_coarse.shape == (1, H // 2, W // 2, C)
    f32, bf16 = jnp.float32, jnp.bfloat16
    npair = H // 2
    npair2 = npair - M1
    nj = M1 + D
    nsem = D + 1
    nct = W // MT
    nqt = (W // 2) // MT
    na = H * W // S
    nwin = S // TW
    nwt = (na // TH) * nwin
    rest0 = INIT + PER * npair2
    assert W % MT == 0 and (W // 2) % MT == 0 and NRING > D
    assert (H * W) % S == 0 and na % TH == 0 and S % TW == 0
    assert nwin % PER == 0 and INIT % PER == 0 and rest0 <= nwt

    def pairs_needed(t):
        return -(-((t // nwin + 1) * TH * S) // (2 * W))

    assert pairs_needed(INIT - 1) <= M1
    assert all(pairs_needed(INIT + PER * (m + 1) - 1) <= M1 + m for m in range(npair2))

    def kernel(c_hbm, p_hbm, wl_hbm, wo_hbm, o_hbm,
               buf, pbuf, wl_v, wo_v, wf_v, jsem, wsem, osem, bsem, tsem):
        copy = pltpu.make_async_copy
        buf_w = buf.reshape(na, S, C)

        def pidx(m):
            if isinstance(m, int):
                return m % NRING if m < M1 else NRING + m - M1
            return jnp.where(m < M1, m % NRING, NRING + m - M1)

        def c_piece(m, k):
            at = (2 * m + k // nct, pl.ds((k % nct) * MT, MT))
            return copy(c_hbm.at[at], buf.at[at], jsem.at[m % nsem])

        def p_piece(m, k):
            px = pl.ds(k * MT, MT)
            return copy(p_hbm.at[m, px], pbuf.at[pidx(m), px], jsem.at[m % nsem])

        def wait_pair(m):
            rows = pl.ds(2 * m, 2)
            copy(c_hbm.at[rows], buf.at[rows], jsem.at[m % nsem]).wait()
            copy(p_hbm.at[m], pbuf.at[pidx(m)], jsem.at[m % nsem]).wait()

        def background():
            rows = pl.ds(2 * nj, H - 2 - 2 * nj)
            head = (H - 2, pl.ds(0, W - TAIL))
            return [
                copy(p_hbm.at[pl.ds(nj, npair - nj)],
                     pbuf.at[pl.ds(NRING + D, npair - nj)], bsem.at[0]),
                copy(c_hbm.at[rows], buf.at[rows], bsem.at[0]),
                copy(c_hbm.at[head], buf.at[head], bsem.at[0]),
            ]

        def background_tail():
            part = (H - 2, pl.ds(W - TAIL, TAIL))
            return [
                copy(c_hbm.at[part], buf.at[part], tsem.at[0]),
                copy(c_hbm.at[H - 1], buf.at[H - 1], tsem.at[0]),
            ]

        def start_write(a0, w0):
            win = (pl.ds(a0, TH), pl.ds(w0, TW))
            copy(buf_w.at[win], o_hbm.at[win], osem.at[0]).start()

        wl_cp = copy(wl_hbm, wl_v, wsem.at[0])
        wo_cp = copy(wo_hbm, wo_v, wsem.at[0])
        wl_cp.start()
        wo_cp.start()

        def first(m, carry):
            for k in range(nqt):
                p_piece(m, k).start()
            for k in range(2 * nct):
                c_piece(m, k).start()
            return carry

        jax.lax.fori_loop(0, D, first, 0)
        for cp in background() + background_tail():
            cp.start(priority=1)

        wl_cp.wait()
        wo_cp.wait()
        wf_v[...] = jnp.dot(wl_v[...], wo_v[...], preferred_element_type=f32).astype(bf16)

        def row_pair(m, after_q, after_c):
            ups = []
            for i in range(nqt):
                q = jnp.dot(pbuf[pidx(m), pl.ds(i * MT, MT), :], wo_v[...],
                            preferred_element_type=f32)
                u = pltpu.bitcast(q.astype(bf16).astype(f32), jnp.uint32)
                ups.append(pltpu.bitcast(u | (u >> 16), bf16))
            for i in range(nqt):
                after_q(i, ups[i])
            up = jnp.concatenate(ups, axis=0).astype(f32)

            def at(t):
                return (2 * m + t // nct, pl.ds((t % nct) * MT, MT), slice(None))

            def mm(t):
                return jnp.dot(buf[at(t)], wf_v[...], preferred_element_type=f32)

            nt = 2 * nct
            accs = [mm(t) for t in range(LAG)]
            for t in range(nt):
                if t + LAG < nt:
                    accs.append(mm(t + LAG))
                lo = (t % nct) * MT
                buf[at(t)] = (accs[t] + up[lo:lo + MT]).astype(bf16)
                after_c(t)

        def body1(m, carry):
            wait_pair(m)

            def after_q(i, val):
                pbuf[pidx(m + D), pl.ds(i * MT, 16), pl.ds(0, 128)] = val[0:16, 0:128]
                p_piece(m + D, i).start()

            row_pair(m, after_q, lambda t: c_piece(m + D, t).start())
            return carry

        jax.lax.fori_loop(0, M1, body1, 0)

        for m in range(M1, nj):
            wait_pair(m)
        for cp in background():
            cp.wait()
        for t in range(INIT):
            start_write((t // nwin) * TH, (t % nwin) * TW)
        for cp in background_tail():
            cp.wait()

        def body2(m, carry):
            g = m + INIT // PER
            a0 = (g // (nwin // PER)) * TH
            w0 = (g % (nwin // PER)) * (PER * TW)
            nt = 2 * nct
            lead = PER - nt

            def wr(k):
                start_write(a0, pl.multiple_of(w0 + k * TW, TW))

            for k in range(lead):
                wr(k)
            row_pair(M1 + m, lambda i, val: None, lambda t: wr(lead + t))
            return carry

        jax.lax.fori_loop(0, npair2, body2, 0)
        for t in range(rest0, nwt):
            start_write((t // nwin) * TH, (t % nwin) * TW)
        copy(buf_w, o_hbm, osem.at[0]).wait()

    out = pl.pallas_call(
        kernel,
        in_specs=[pl.BlockSpec(memory_space=pl.ANY)] * 4,
        out_specs=pl.BlockSpec(memory_space=pl.ANY),
        out_shape=jax.ShapeDtypeStruct((na, S, C), c_fine.dtype),
        scratch_shapes=[
            pltpu.VMEM((H, W, C), bf16),
            pltpu.VMEM((NRING + npair2, W // 2, C), bf16),
            pltpu.VMEM((C, C), bf16),
            pltpu.VMEM((C, C), bf16),
            pltpu.VMEM((C, C), bf16),
            pltpu.SemaphoreType.DMA((nsem,)),
            pltpu.SemaphoreType.DMA((1,)),
            pltpu.SemaphoreType.DMA((1,)),
            pltpu.SemaphoreType.DMA((1,)),
            pltpu.SemaphoreType.DMA((1,)),
        ],
        compiler_params=pltpu.CompilerParams(
            vmem_limit_bytes=127 * 1024 * 1024,
            disable_bounds_checks=True,
        ),
    )(
        c_fine.reshape(H, W, C),
        p_coarse.reshape(H // 2, W // 2, C),
        w_lat,
        w_out.reshape(C, C),
    )
    return out.reshape(B, H, W, C)
```

```python
import jax
import jax.numpy as jnp
import jax.experimental.pallas as pl
import jax.experimental.pallas.tpu as pltpu

M1 = 109
D = 2
NRING = 4
MT = 64
LAG = 2
DELAY = (2, 0, 8, 10)
S = 2048
TH = 6
TW = 16
INIT = 64
PER = 16
TAIL = 256


@jax.jit
def pallas_standalone__detection_seg_fpn_lateral__vision_kernel(
    c_fine: jax.Array,
    p_coarse: jax.Array,
    w_lat: jax.Array,
    w_out: jax.Array,
):
    B, H, W, C = c_fine.shape
    assert B == 1 and w_out.shape == (1, 1, C, C)
    assert p_coarse.shape == (1, H // 2, W // 2, C)
    f32, bf16 = jnp.float32, jnp.bfloat16
    npair = H // 2
    npair2 = npair - M1
    nj = M1 + D
    nsem = D + 1
    nct = W // MT
    nqt = (W // 2) // MT
    nt = 2 * nct
    na = H * W // S
    nwin = S // TW
    nwt = (na // TH) * nwin
    rest0 = INIT + PER * npair2
    assert W % MT == 0 and (W // 2) % MT == 0 and NRING > D and len(DELAY) == nqt + 1
    assert (H * W) % S == 0 and na % TH == 0 and S % TW == 0
    assert nwin % PER == 0 and INIT % PER == 0 and rest0 <= nwt and PER >= nt

    def pairs_needed(t):
        return -(-((t // nwin + 1) * TH * S) // (2 * W))

    assert pairs_needed(INIT - 1) <= M1
    assert all(pairs_needed(INIT + PER * (m + 1) - 1) <= M1 + m for m in range(npair2))

    def kernel(c_hbm, p_hbm, wl_hbm, wo_hbm, o_hbm,
               buf, pbuf, wl_v, wo_v, wf_v, csem, psem, wsem, osem, bsem, tsem):
        copy = pltpu.make_async_copy
        buf_w = buf.reshape(na, S, C)

        def pidx(m):
            if isinstance(m, int):
                return m % NRING if m < M1 else NRING + m - M1
            return jnp.where(m < M1, m % NRING, NRING + m - M1)

        def c_piece(m, k):
            at = (2 * m + k // nct, pl.ds((k % nct) * MT, MT))
            return copy(c_hbm.at[at], buf.at[at], csem.at[m % nsem])

        def p_piece(m, k):
            px = pl.ds(k * MT, MT)
            return copy(p_hbm.at[m, px], pbuf.at[pidx(m), px], psem.at[m % nsem])

        def wait_pair(m):
            rows = pl.ds(2 * m, 2)
            copy(p_hbm.at[m], pbuf.at[pidx(m)], psem.at[m % nsem]).wait()
            copy(c_hbm.at[rows], buf.at[rows], csem.at[m % nsem]).wait()

        def background():
            rows = pl.ds(2 * nj, H - 2 - 2 * nj)
            head = (H - 2, pl.ds(0, W - TAIL))
            return [
                copy(p_hbm.at[pl.ds(nj, npair - nj)],
                     pbuf.at[pl.ds(NRING + D, npair - nj)], bsem.at[0]),
                copy(c_hbm.at[rows], buf.at[rows], bsem.at[0]),
                copy(c_hbm.at[head], buf.at[head], bsem.at[0]),
            ]

        def background_tail():
            part = (H - 2, pl.ds(W - TAIL, TAIL))
            return [
                copy(c_hbm.at[part], buf.at[part], tsem.at[0]),
                copy(c_hbm.at[H - 1], buf.at[H - 1], tsem.at[0]),
            ]

        def start_write(a0, w0):
            win = (pl.ds(a0, TH), pl.ds(w0, TW))
            copy(buf_w.at[win], o_hbm.at[win], osem.at[0]).start()

        wl_cp = copy(wl_hbm, wl_v, wsem.at[0])
        wo_cp = copy(wo_hbm, wo_v, wsem.at[0])
        wl_cp.start()
        wo_cp.start()

        def first(m, carry):
            for k in range(nqt):
                p_piece(m, k).start()
            for k in range(nt):
                c_piece(m, k).start()
            return carry

        jax.lax.fori_loop(0, D, first, 0)
        for cp in background() + background_tail():
            cp.start(priority=1)

        wl_cp.wait()
        wo_cp.wait()
        wf_v[...] = jnp.dot(wl_v[...], wo_v[...], preferred_element_type=f32).astype(bf16)

        def row_pair(m, prefetch, after_tile):
            def start_after(piece, dst, val, delay):
                val = val[0:16, 0:128]
                for _ in range(delay):
                    val = val * 1.0001 + 1.0
                dst[...] = val.astype(bf16)
                piece.start()

            def p_dst(k):
                return pbuf.at[pidx(m + D), pl.ds(k * MT, 16), pl.ds(0, 128)]

            ups = []
            for i in range(nqt):
                x = pbuf[pidx(m), pl.ds(i * MT, MT), :]
                q = jnp.dot(x, wo_v[...], preferred_element_type=f32)
                if prefetch and i == 0:
                    start_after(p_piece(m + D, 0), p_dst(0), x.astype(f32), DELAY[0])
                u = pltpu.bitcast(q.astype(bf16).astype(f32), jnp.uint32)
                ups.append(pltpu.bitcast(u | (u >> 16), bf16).astype(f32))
            if prefetch:
                for i in range(1, nqt):
                    start_after(p_piece(m + D, i), p_dst(i), ups[i - 1], DELAY[i])
            up = jnp.concatenate(ups, axis=0)

            def at(t):
                return (2 * m + t // nct, pl.ds((t % nct) * MT, MT), slice(None))

            def mm(t):
                return jnp.dot(buf[at(t)], wf_v[...], preferred_element_type=f32)

            accs = [mm(t) for t in range(LAG)]
            if prefetch:
                dst = buf.at[2 * (m + D), pl.ds(0, 16), pl.ds(0, 128)]
                start_after(c_piece(m + D, 0), dst, ups[-1], DELAY[nqt])
            for t in range(nt):
                if t + LAG < nt:
                    accs.append(mm(t + LAG))
                lo = (t % nct) * MT
                buf[at(t)] = (accs[t] + up[lo:lo + MT]).astype(bf16)
                after_tile(t)

        def body1(m, carry):
            wait_pair(m)

            def after_tile(t):
                if t + 1 < nt:
                    c_piece(m + D, t + 1).start()

            row_pair(m, True, after_tile)
            return carry

        jax.lax.fori_loop(0, M1, body1, 0)

        for m in range(M1, nj):
            wait_pair(m)
        for cp in background():
            cp.wait()
        for t in range(INIT):
            start_write((t // nwin) * TH, (t % nwin) * TW)
        for cp in background_tail():
            cp.wait()

        def body2(m, carry):
            g = m + INIT // PER
            a0 = (g // (nwin // PER)) * TH
            w0 = (g % (nwin // PER)) * (PER * TW)

            def wr(k):
                start_write(a0, pl.multiple_of(w0 + k * TW, TW))

            for k in range(PER - nt):
                wr(k)
            row_pair(M1 + m, False, lambda t: wr(PER - nt + t))
            return carry

        jax.lax.fori_loop(0, npair2, body2, 0)
        for t in range(rest0, nwt):
            start_write((t // nwin) * TH, (t % nwin) * TW)
        copy(buf_w, o_hbm, osem.at[0]).wait()

    out = pl.pallas_call(
        kernel,
        in_specs=[pl.BlockSpec(memory_space=pl.ANY)] * 4,
        out_specs=pl.BlockSpec(memory_space=pl.ANY),
        out_shape=jax.ShapeDtypeStruct((na, S, C), c_fine.dtype),
        scratch_shapes=[
            pltpu.VMEM((H, W, C), bf16),
            pltpu.VMEM((NRING + npair2, W // 2, C), bf16),
            pltpu.VMEM((C, C), bf16),
            pltpu.VMEM((C, C), bf16),
            pltpu.VMEM((C, C), bf16),
            pltpu.SemaphoreType.DMA((nsem,)),
            pltpu.SemaphoreType.DMA((nsem,)),
            pltpu.SemaphoreType.DMA((1,)),
            pltpu.SemaphoreType.DMA((1,)),
            pltpu.SemaphoreType.DMA((1,)),
            pltpu.SemaphoreType.DMA((1,)),
        ],
        compiler_params=pltpu.CompilerParams(vmem_limit_bytes=127 * 1024 * 1024),
    )(
        c_fine.reshape(H, W, C),
        p_coarse.reshape(H // 2, W // 2, C),
        w_lat,
        w_out.reshape(C, C),
    )
    return out.reshape(B, H, W, C)
```

```python
import jax
import jax.numpy as jnp
import jax.experimental.pallas as pl
import jax.experimental.pallas.tpu as pltpu

M1 = 108
D = 2
NRING = 4
MT = 64
LAG = 2
DELAY = (2, 0, 8, 10)
S = 2048
TH = 6
TW = 16
INIT = 64
PER = 16
U2 = 2
TAIL = 256


@jax.jit
def pallas_standalone__detection_seg_fpn_lateral__vision_kernel(
    c_fine: jax.Array,
    p_coarse: jax.Array,
    w_lat: jax.Array,
    w_out: jax.Array,
):
    B, H, W, C = c_fine.shape
    assert B == 1 and w_out.shape == (1, 1, C, C)
    assert p_coarse.shape == (1, H // 2, W // 2, C)
    f32, bf16 = jnp.float32, jnp.bfloat16
    npair = H // 2
    npair2 = npair - M1
    nj = M1 + D
    nsem = D + 1
    nct = W // MT
    nqt = (W // 2) // MT
    nt = 2 * nct
    na = H * W // S
    nwin = S // TW
    nwt = (na // TH) * nwin
    rest0 = INIT + PER * npair2
    assert W % MT == 0 and (W // 2) % MT == 0 and NRING > D and len(DELAY) == nqt + 1
    assert (H * W) % S == 0 and na % TH == 0 and S % TW == 0
    assert nwin % PER == 0 and INIT % PER == 0 and rest0 <= nwt and PER >= nt
    assert npair2 % U2 == 0

    def pairs_needed(t):
        return -(-((t // nwin + 1) * TH * S) // (2 * W))

    assert pairs_needed(INIT - 1) <= M1
    assert all(pairs_needed(INIT + PER * (m + 1) - 1) <= M1 + m for m in range(npair2))

    def kernel(c_hbm, p_hbm, wl_hbm, wo_hbm, o_hbm,
               buf, pbuf, wl_v, wo_v, wf_v, csem, psem, wsem, osem, bsem, tsem):
        copy = pltpu.make_async_copy
        buf_w = buf.reshape(na, S, C)

        def pidx(m):
            if isinstance(m, int):
                return m % NRING if m < M1 else NRING + m - M1
            return jnp.where(m < M1, m % NRING, NRING + m - M1)

        def c_piece(m, k):
            at = (2 * m + k // nct, pl.ds((k % nct) * MT, MT))
            return copy(c_hbm.at[at], buf.at[at], csem.at[m % nsem])

        def p_piece(m, k):
            px = pl.ds(k * MT, MT)
            return copy(p_hbm.at[m, px], pbuf.at[pidx(m), px], psem.at[m % nsem])

        def wait_pair(m):
            rows = pl.ds(2 * m, 2)
            copy(p_hbm.at[m], pbuf.at[pidx(m)], psem.at[m % nsem]).wait()
            copy(c_hbm.at[rows], buf.at[rows], csem.at[m % nsem]).wait()

        def background():
            rows = pl.ds(2 * nj, H - 2 - 2 * nj)
            head = (H - 2, pl.ds(0, W - TAIL))
            return [
                copy(p_hbm.at[pl.ds(nj, npair - nj)],
                     pbuf.at[pl.ds(NRING + D, npair - nj)], bsem.at[0]),
                copy(c_hbm.at[rows], buf.at[rows], bsem.at[0]),
                copy(c_hbm.at[head], buf.at[head], bsem.at[0]),
            ]

        def background_tail():
            part = (H - 2, pl.ds(W - TAIL, TAIL))
            return [
                copy(c_hbm.at[part], buf.at[part], tsem.at[0]),
                copy(c_hbm.at[H - 1], buf.at[H - 1], tsem.at[0]),
            ]

        def start_write(a0, w0):
            win = (pl.ds(a0, TH), pl.ds(w0, TW))
            copy(buf_w.at[win], o_hbm.at[win], osem.at[0]).start()

        wl_cp = copy(wl_hbm, wl_v, wsem.at[0])
        wo_cp = copy(wo_hbm, wo_v, wsem.at[0])
        wl_cp.start()
        wo_cp.start()

        def first(m, carry):
            for k in range(nqt):
                p_piece(m, k).start()
            for k in range(nt):
                c_piece(m, k).start()
            return carry

        jax.lax.fori_loop(0, D, first, 0)
        for cp in background() + background_tail():
            cp.start(priority=1)

        wl_cp.wait()
        wo_cp.wait()
        wf_v[...] = jnp.dot(wl_v[...], wo_v[...], preferred_element_type=f32).astype(bf16)

        def row_pair(m, prefetch, after_tile):
            def start_after(piece, dst, val, delay):
                val = val[0:16, 0:128]
                for _ in range(delay):
                    val = val * 1.0001 + 1.0
                dst[...] = val.astype(bf16)
                piece.start()

            def p_dst(k):
                return pbuf.at[pidx(m + D), pl.ds(k * MT, 16), pl.ds(0, 128)]

            ups = []
            for i in range(nqt):
                x = pbuf[pidx(m), pl.ds(i * MT, MT), :]
                q = jnp.dot(x, wo_v[...], preferred_element_type=f32)
                if prefetch and i == 0:
                    start_after(p_piece(m + D, 0), p_dst(0), x.astype(f32), DELAY[0])
                u = pltpu.bitcast(q.astype(bf16).astype(f32), jnp.uint32)
                ups.append(pltpu.bitcast(u | (u >> 16), bf16).astype(f32))
            if prefetch:
                for i in range(1, nqt):
                    start_after(p_piece(m + D, i), p_dst(i), ups[i - 1], DELAY[i])
            up = jnp.concatenate(ups, axis=0)

            def at(t):
                return (2 * m + t // nct, pl.ds((t % nct) * MT, MT), slice(None))

            def mm(t):
                return jnp.dot(buf[at(t)], wf_v[...], preferred_element_type=f32)

            accs = [mm(t) for t in range(LAG)]
            if prefetch:
                dst = buf.at[2 * (m + D), pl.ds(0, 16), pl.ds(0, 128)]
                start_after(c_piece(m + D, 0), dst, ups[-1], DELAY[nqt])
            for t in range(nt):
                if t + LAG < nt:
                    accs.append(mm(t + LAG))
                lo = (t % nct) * MT
                buf[at(t)] = (accs[t] + up[lo:lo + MT]).astype(bf16)
                after_tile(t)

        def body1(m, carry):
            wait_pair(m)

            def after_tile(t):
                if t + 1 < nt:
                    c_piece(m + D, t + 1).start()

            row_pair(m, True, after_tile)
            return carry

        jax.lax.fori_loop(0, M1, body1, 0)

        for m in range(M1, nj):
            wait_pair(m)
        for cp in background():
            cp.wait()
        for t in range(INIT):
            start_write((t // nwin) * TH, (t % nwin) * TW)
        for cp in background_tail():
            cp.wait()

        def pair2(m):
            g = m + INIT // PER
            a0 = (g // (nwin // PER)) * TH
            w0 = (g % (nwin // PER)) * (PER * TW)

            def wr(k):
                start_write(a0, pl.multiple_of(w0 + k * TW, TW))

            for k in range(PER - nt):
                wr(k)
            row_pair(M1 + m, False, lambda t: wr(PER - nt + t))

        def body2(i, carry):
            for u in range(U2):
                pair2(i * U2 + u)
            return carry

        jax.lax.fori_loop(0, npair2 // U2, body2, 0)
        for t in range(rest0, nwt):
            start_write((t // nwin) * TH, (t % nwin) * TW)
        copy(buf_w, o_hbm, osem.at[0]).wait()

    out = pl.pallas_call(
        kernel,
        in_specs=[pl.BlockSpec(memory_space=pl.ANY)] * 4,
        out_specs=pl.BlockSpec(memory_space=pl.ANY),
        out_shape=jax.ShapeDtypeStruct((na, S, C), c_fine.dtype),
        scratch_shapes=[
            pltpu.VMEM((H, W, C), bf16),
            pltpu.VMEM((NRING + npair2, W // 2, C), bf16),
            pltpu.VMEM((C, C), bf16),
            pltpu.VMEM((C, C), bf16),
            pltpu.VMEM((C, C), bf16),
            pltpu.SemaphoreType.DMA((nsem,)),
            pltpu.SemaphoreType.DMA((nsem,)),
            pltpu.SemaphoreType.DMA((1,)),
            pltpu.SemaphoreType.DMA((1,)),
            pltpu.SemaphoreType.DMA((1,)),
            pltpu.SemaphoreType.DMA((1,)),
        ],
        compiler_params=pltpu.CompilerParams(vmem_limit_bytes=127 * 1024 * 1024),
    )(
        c_fine.reshape(H, W, C),
        p_coarse.reshape(H // 2, W // 2, C),
        w_lat,
        w_out.reshape(C, C),
    )
    return out.reshape(B, H, W, C)
```

```python
import jax
import jax.numpy as jnp
import jax.experimental.pallas as pl
import jax.experimental.pallas.tpu as pltpu

G = 4
TW0 = 16
NE = 112
LEADG = 2
NR = 4
S = 2048
TH1, TW1 = 6, 8
THP, TWP = 4, 8
N1C, N1P = 11, 4
PRE1C, PRE1P = 116, 48
NSAT = 28
WSPLIT = 70
NTAIL = 14
TH, TW = 6, 16
INIT = 64
PER = 16
U2 = 2
MT = 64
LAG = 2


def _weave(xs, ys):
    out, i, j = [], 0, 0
    while i < len(xs) or j < len(ys):
        if j < len(ys) and j * len(xs) <= i * len(ys):
            out.append(ys[j])
            j += 1
        else:
            out.append(xs[i])
            i += 1
    return out


def _div(i, n, limit):
    if isinstance(i, int) or n & (n - 1) == 0:
        return i // n
    magic = -(-(1 << 18) // n)
    assert limit * magic < 2**31 and all((x * magic) >> 18 == x // n for x in range(limit))
    return (i * magic) >> 18


def _aligned(x, k):
    return x if isinstance(x, int) else pl.multiple_of(x, k)


@jax.jit
def pallas_standalone__detection_seg_fpn_lateral__vision_kernel(
    c_fine: jax.Array,
    p_coarse: jax.Array,
    w_lat: jax.Array,
    w_out: jax.Array,
):
    B, H, W, C = c_fine.shape
    assert B == 1 and w_out.shape == (1, 1, C, C)
    assert p_coarse.shape == (1, H // 2, W // 2, C)
    f32, bf16 = jnp.float32, jnp.bfloat16
    npair, pw, pc = H // 2, 2 * W, W // 2
    pg = G * pc
    ng, neg = npair // G, NE // G
    nlg = ng - neg
    nig = neg - LEADG
    m1 = nig * G
    na = H * W // S
    assert npair % G == 0 and NE % G == 0 and NR > LEADG and (H * W) % S == 0
    px0, nw0 = G * TW0, pw // TW0
    n0c, n0p = nw0 // G, pc // px0
    assert pw % TW0 == 0 and nw0 % G == 0 and pc % px0 == 0
    a1, nw1, nwp = NE * pw // S, S // TW1, pg // TWP
    assert (NE * pw) % S == 0 and (na - a1) % TH1 == 0 and S % TW1 == 0
    assert nlg % THP == 0 and pg % TWP == 0
    n1c, n1p = (na - a1) // TH1 * nw1, nlg // THP * nwp
    post1c, post1p = n1c - PRE1C - m1 * N1C, n1p - PRE1P - m1 * N1P
    assert NTAIL <= post1c and NTAIL < nw1 and post1p >= 0
    nwin = S // TW
    nwt = na // TH * nwin
    nb2 = min(npair - m1, (nwt - nwin - INIT) // PER) // U2
    rest0 = INIT + PER * nb2 * U2
    assert na % TH == 0 and S % TW == 0 and nwin % PER == 0 and INIT % PER == 0

    def pairs_needed(t):
        return -(-((t // nwin + 1) * TH * S) // pw)

    assert pairs_needed(INIT - 1) <= m1
    assert all(pairs_needed(INIT + PER * (k + 1) - 1) <= m1 + k for k in range(nb2 * U2))
    nt, nq = pw // MT, pc // MT
    assert pc % MT == 0 and W % MT == 0
    CS, PS, LC, LP, WT, TL, OUT = 0, NR, 2 * NR, 2 * NR + 1, 2 * NR + 2, 2 * NR + 3, 2 * NR + 4

    def kernel(c_pair, c_s, p_g, wl_hbm, wo_hbm, o_hbm, buf, pbuf, wl_v, wo_v, wf_v, sem):
        copy = pltpu.make_async_copy
        buf_s = buf.reshape(na, S, C)

        def early_c(g, k):
            at = (pl.ds(g * G, G), pl.ds(_aligned(k * TW0, TW0), TW0))
            return copy(c_pair.at[at], buf.at[at], sem.at[CS + g % NR])

        def early_p(g, k):
            px = pl.ds(_aligned(k * px0, px0), px0)
            return copy(p_g.at[g, px], pbuf.at[g % NR, px], sem.at[PS + g % NR])

        def wait_group(g):
            copy(p_g.at[g], pbuf.at[g % NR], sem.at[PS + g % NR]).wait()
            pairs = pl.ds(g * G, G)
            copy(c_pair.at[pairs], buf.at[pairs], sem.at[CS + g % NR]).wait()

        def late_c(i, s=LC):
            q = _div(i, nw1, n1c)
            at = (pl.ds(a1 + q * TH1, TH1), pl.ds(_aligned((i - q * nw1) * TW1, TW1), TW1))
            return copy(c_s.at[at], buf_s.at[at], sem.at[s])

        def late_p(i):
            q = _div(i, nwp, n1p)
            px = pl.ds(_aligned((i - q * nwp) * TWP, TWP), TWP)
            return copy(p_g.at[pl.ds(neg + q * THP, THP), px],
                        pbuf.at[pl.ds(NR + q * THP, THP), px], sem.at[LP])

        def start_write(a0, w0):
            win = (pl.ds(a0, TH), pl.ds(w0, TW))
            copy(buf_s.at[win], o_hbm.at[win], sem.at[OUT]).start()

        def writes(i, n):
            a0 = (i // (nwin // n)) * TH
            w0 = (i % (nwin // n)) * (n * TW)
            return [lambda k=k: start_write(a0, pl.multiple_of(w0 + k * TW, TW)) for k in range(n)]

        def queue_writes(lo, hi):
            def body(i, carry):
                for start in writes(i, 4):
                    start()
                return carry

            jax.lax.fori_loop(lo // 4, hi // 4, body, 0)

        def high(fn, *args):
            return lambda: fn(*args).start()

        def low(fn, *args):
            return lambda: fn(*args).start(priority=1)

        wl_cp = copy(wl_hbm, wl_v, sem.at[WT])
        wo_cp = copy(wo_hbm, wo_v, sem.at[WT])
        wl_cp.start()
        wo_cp.start()
        lows = _weave([low(late_c, i) for i in range(PRE1C)],
                      [low(late_p, i) for i in range(PRE1P)])
        highs = []
        for g in range(LEADG):
            highs += _weave([high(early_c, g, k) for k in range(nw0)],
                            [high(early_p, g, k) for k in range(G * n0p)])
        starts = lows[:NSAT] + _weave(highs, lows[NSAT:])
        for start in starts[:WSPLIT]:
            start()
        wl_cp.wait()
        wo_cp.wait()
        wf_v[...] = jnp.dot(wl_v[...], wo_v[...], preferred_element_type=f32).astype(bf16)
        for start in starts[WSPLIT:]:
            start()

        def pair(m, slot, j, starts=()):
            ups = []
            for i in range(nq):
                x = pbuf[slot, pl.ds(_aligned(j * pc + i * MT, MT), MT), :]
                q = jnp.dot(x, wo_v[...], preferred_element_type=f32)
                u = pltpu.bitcast(q.astype(bf16).astype(f32), jnp.uint32)
                ups.append(pltpu.bitcast(u | (u >> 16), bf16).astype(f32))
            up = jnp.concatenate(ups, axis=0)

            def mm(t):
                return jnp.dot(buf[m, pl.ds(t * MT, MT), :], wf_v[...],
                               preferred_element_type=f32)

            accs = [mm(t) for t in range(LAG)]
            for t in range(nt):
                if t + LAG < nt:
                    accs.append(mm(t + LAG))
                lo = (t * MT) % W
                buf[m, pl.ds(t * MT, MT), :] = (accs[t] + up[lo:lo + MT]).astype(bf16)
                for start in starts[t * len(starts) // nt:(t + 1) * len(starts) // nt]:
                    start()

        def group(g, carry):
            wait_group(g)

            def body(j, c2):
                m = g * G + j
                highs = _weave(
                    [high(early_c, g + LEADG, j * n0c + k) for k in range(n0c)],
                    [high(early_p, g + LEADG, j * n0p + k) for k in range(n0p)])
                lows = _weave(
                    [low(late_c, PRE1C + m * N1C + k) for k in range(N1C)],
                    [low(late_p, PRE1P + m * N1P + k) for k in range(N1P)])
                pair(m, g % NR, j, _weave(highs, lows))
                return c2

            jax.lax.fori_loop(0, G, body, 0)
            return carry

        jax.lax.fori_loop(0, nig, group, 0)

        rest = _weave([(late_c, i) for i in range(n1c - post1c, n1c - NTAIL)],
                      [(late_p, i) for i in range(n1p - post1p, n1p)])
        for n, (fn, i) in enumerate(rest):
            fn(i).start(priority=(n + 1) % 2)
        for i in range(n1c - NTAIL, n1c):
            late_c(i, TL).start(priority=1)

        for g in range(nig, neg):
            wait_group(g)
        copy(p_g.at[pl.ds(neg, nlg)], pbuf.at[pl.ds(NR, nlg)], sem.at[LP]).wait()
        body_rows = pl.ds(a1, na - a1 - TH1)
        head = (pl.ds(na - TH1, TH1), pl.ds(0, S - NTAIL * TW1))
        tail = (pl.ds(na - TH1, TH1), pl.ds(S - NTAIL * TW1, NTAIL * TW1))
        copy(c_s.at[body_rows], buf_s.at[body_rows], sem.at[LC]).wait()
        copy(c_s.at[head], buf_s.at[head], sem.at[LC]).wait()
        queue_writes(0, INIT)
        copy(c_s.at[tail], buf_s.at[tail], sem.at[TL]).wait()

        def pair2(m, starts=()):
            g = m // G
            pair(m, jnp.where(g < neg, g % NR, NR + g - neg), m % G, starts)

        def body2(i, carry):
            for u in range(U2):
                k = i * U2 + u
                pair2(m1 + k, writes(k + INIT // PER, PER))
            return carry

        def body3(m, carry):
            pair2(m)
            return carry

        jax.lax.fori_loop(0, nb2, body2, 0)
        jax.lax.fori_loop(m1 + nb2 * U2, npair, body3, 0)
        queue_writes(rest0, nwt)
        copy(buf_s, o_hbm, sem.at[OUT]).wait()

    out = pl.pallas_call(
        kernel,
        in_specs=[pl.BlockSpec(memory_space=pl.ANY)] * 5,
        out_specs=pl.BlockSpec(memory_space=pl.ANY),
        out_shape=jax.ShapeDtypeStruct((na, S, C), c_fine.dtype),
        scratch_shapes=[
            pltpu.VMEM((npair, pw, C), bf16),
            pltpu.VMEM((NR + nlg, pg, C), bf16),
            pltpu.VMEM((C, C), bf16),
            pltpu.VMEM((C, C), bf16),
            pltpu.VMEM((C, C), bf16),
            pltpu.SemaphoreType.DMA((OUT + 1,)),
        ],
        compiler_params=pltpu.CompilerParams(
            vmem_limit_bytes=127 * 1024 * 1024,
            disable_bounds_checks=True,
        ),
    )(
        c_fine.reshape(npair, pw, C),
        c_fine.reshape(na, S, C),
        p_coarse.reshape(ng, pg, C),
        w_lat,
        w_out.reshape(C, C),
    )
    return out.reshape(B, H, W, C)
```

```python
import jax
import jax.numpy as jnp
import jax.experimental.pallas as pl
import jax.experimental.pallas.tpu as pltpu

G = 4
TW0 = 16
NE = 112
LEADG = 2
NR = 4
S = 2048
TH1, TW1 = 6, 8
THP, TWP = 4, 8
N1C, N1P = 11, 4
PRE1C, PRE1P = 116, 48
NSAT = 28
WSPLIT = 70
NTAIL = 14
TH, TW = 6, 16
INIT = 32
PER = 16
U1 = 2
U2 = 2
MT = 64
LAG = 2


def _weave(xs, ys):
    out, i, j = [], 0, 0
    while i < len(xs) or j < len(ys):
        if j < len(ys) and j * len(xs) <= i * len(ys):
            out.append(ys[j])
            j += 1
        else:
            out.append(xs[i])
            i += 1
    return out


def _div(i, n, limit):
    if isinstance(i, int) or n & (n - 1) == 0:
        return i // n
    magic = -(-(1 << 18) // n)
    assert limit * magic < 2**31 and all((x * magic) >> 18 == x // n for x in range(limit))
    return (i * magic) >> 18


def _aligned(x, k):
    return x if isinstance(x, int) else pl.multiple_of(x, k)


@jax.jit
def pallas_standalone__detection_seg_fpn_lateral__vision_kernel(
    c_fine: jax.Array,
    p_coarse: jax.Array,
    w_lat: jax.Array,
    w_out: jax.Array,
):
    B, H, W, C = c_fine.shape
    assert B == 1 and w_out.shape == (1, 1, C, C)
    assert p_coarse.shape == (1, H // 2, W // 2, C)
    f32, bf16 = jnp.float32, jnp.bfloat16
    npair, pw, pc = H // 2, 2 * W, W // 2
    pg = G * pc
    ng, neg = npair // G, NE // G
    nlg = ng - neg
    nig = neg - LEADG
    m1 = nig * G
    na = H * W // S
    assert npair % G == 0 and NE % G == 0 and G % U1 == 0 and NR > LEADG and (H * W) % S == 0
    px0, nw0 = G * TW0, pw // TW0
    n0c, n0p = nw0 // G, pc // px0
    assert pw % TW0 == 0 and nw0 % G == 0 and pc % px0 == 0
    a1, nw1, nwp = NE * pw // S, S // TW1, pg // TWP
    assert (NE * pw) % S == 0 and (na - a1) % TH1 == 0 and S % TW1 == 0
    assert nlg % THP == 0 and pg % TWP == 0
    n1c, n1p = (na - a1) // TH1 * nw1, nlg // THP * nwp
    post1c, post1p = n1c - PRE1C - m1 * N1C, n1p - PRE1P - m1 * N1P
    assert NTAIL <= post1c and NTAIL < nw1 and post1p >= 0
    nwin = S // TW
    nwt = na // TH * nwin
    nb2 = min(npair - m1, (nwt - nwin - INIT) // PER) // U2
    rest0 = INIT + PER * nb2 * U2
    assert na % TH == 0 and S % TW == 0 and nwin % PER == 0 and INIT % PER == 0

    def pairs_needed(t):
        return -(-((t // nwin + 1) * TH * S) // pw)

    assert pairs_needed(INIT - 1) <= m1
    assert all(pairs_needed(INIT + PER * (k + 1) - 1) <= m1 + k for k in range(nb2 * U2))
    nt, nq = pw // MT, pc // MT
    assert pc % MT == 0 and W % MT == 0
    CS, PS, LC, LP, WT, TL, OUT = 0, NR, 2 * NR, 2 * NR + 1, 2 * NR + 2, 2 * NR + 3, 2 * NR + 4

    def kernel(c_pair, c_s, p_g, wl_hbm, wo_hbm, o_hbm, buf, pbuf, wl_v, wo_v, wf_v, sem):
        copy = pltpu.make_async_copy
        buf_s = buf.reshape(na, S, C)

        def early_c(g, k):
            at = (pl.ds(g * G, G), pl.ds(_aligned(k * TW0, TW0), TW0))
            return copy(c_pair.at[at], buf.at[at], sem.at[CS + g % NR])

        def early_p(g, k):
            px = pl.ds(_aligned(k * px0, px0), px0)
            return copy(p_g.at[g, px], pbuf.at[g % NR, px], sem.at[PS + g % NR])

        def wait_group(g):
            copy(p_g.at[g], pbuf.at[g % NR], sem.at[PS + g % NR]).wait()
            pairs = pl.ds(g * G, G)
            copy(c_pair.at[pairs], buf.at[pairs], sem.at[CS + g % NR]).wait()

        def late_c(i, s=LC):
            q = _div(i, nw1, n1c)
            at = (pl.ds(a1 + q * TH1, TH1), pl.ds(_aligned((i - q * nw1) * TW1, TW1), TW1))
            return copy(c_s.at[at], buf_s.at[at], sem.at[s])

        def late_p(i):
            q = _div(i, nwp, n1p)
            px = pl.ds(_aligned((i - q * nwp) * TWP, TWP), TWP)
            return copy(p_g.at[pl.ds(neg + q * THP, THP), px],
                        pbuf.at[pl.ds(NR + q * THP, THP), px], sem.at[LP])

        def start_write(a0, w0):
            win = (pl.ds(a0, TH), pl.ds(w0, TW))
            copy(buf_s.at[win], o_hbm.at[win], sem.at[OUT]).start()

        def writes(i, n):
            a0 = (i // (nwin // n)) * TH
            w0 = (i % (nwin // n)) * (n * TW)
            return [lambda k=k: start_write(a0, pl.multiple_of(w0 + k * TW, TW)) for k in range(n)]

        def queue_writes(lo, hi):
            def body(i, carry):
                for start in writes(i, 4):
                    start()
                return carry

            jax.lax.fori_loop(lo // 4, hi // 4, body, 0)

        def high(fn, *args):
            return lambda: fn(*args).start()

        def low(fn, *args):
            return lambda: fn(*args).start(priority=1)

        wl_cp = copy(wl_hbm, wl_v, sem.at[WT])
        wo_cp = copy(wo_hbm, wo_v, sem.at[WT])
        wl_cp.start()
        wo_cp.start()
        lows = _weave([low(late_c, i) for i in range(PRE1C)],
                      [low(late_p, i) for i in range(PRE1P)])
        highs = []
        for g in range(LEADG):
            highs += _weave([high(early_c, g, k) for k in range(nw0)],
                            [high(early_p, g, k) for k in range(G * n0p)])
        starts = lows[:NSAT] + _weave(highs, lows[NSAT:])
        for start in starts[:WSPLIT]:
            start()
        wl_cp.wait()
        wo_cp.wait()
        wf_v[...] = jnp.dot(wl_v[...], wo_v[...], preferred_element_type=f32).astype(bf16)
        for start in starts[WSPLIT:]:
            start()

        def pair(m, slot, j, starts=()):
            ups = []
            for i in range(nq):
                x = pbuf[slot, pl.ds(_aligned(j * pc + i * MT, MT), MT), :]
                q = jnp.dot(x, wo_v[...], preferred_element_type=f32)
                u = pltpu.bitcast(q.astype(bf16).astype(f32), jnp.uint32)
                ups.append(pltpu.bitcast(u | (u >> 16), bf16).astype(f32))
            up = jnp.concatenate(ups, axis=0)

            def mm(t):
                return jnp.dot(buf[m, pl.ds(t * MT, MT), :], wf_v[...],
                               preferred_element_type=f32)

            accs = [mm(t) for t in range(LAG)]
            for t in range(nt):
                if t + LAG < nt:
                    accs.append(mm(t + LAG))
                lo = (t * MT) % W
                buf[m, pl.ds(t * MT, MT), :] = (accs[t] + up[lo:lo + MT]).astype(bf16)
                for start in starts[t * len(starts) // nt:(t + 1) * len(starts) // nt]:
                    start()

        def group(g, carry):
            wait_group(g)

            def body(jj, c2):
                for u in range(U1):
                    j = jj * U1 + u
                    m = g * G + j
                    highs = _weave(
                        [high(early_c, g + LEADG, j * n0c + k) for k in range(n0c)],
                        [high(early_p, g + LEADG, j * n0p + k) for k in range(n0p)])
                    lows = _weave(
                        [low(late_c, PRE1C + m * N1C + k) for k in range(N1C)],
                        [low(late_p, PRE1P + m * N1P + k) for k in range(N1P)])
                    pair(m, g % NR, j, _weave(highs, lows))
                return c2

            jax.lax.fori_loop(0, G // U1, body, 0)
            return carry

        jax.lax.fori_loop(0, nig, group, 0)

        rest = _weave([(late_c, i) for i in range(n1c - post1c, n1c - NTAIL)],
                      [(late_p, i) for i in range(n1p - post1p, n1p)])
        for n, (fn, i) in enumerate(rest):
            fn(i).start(priority=(n + 1) % 2)
        for i in range(n1c - NTAIL, n1c):
            late_c(i, TL).start(priority=1)

        for g in range(nig, neg):
            wait_group(g)
        copy(p_g.at[pl.ds(neg, nlg)], pbuf.at[pl.ds(NR, nlg)], sem.at[LP]).wait()
        body_rows = pl.ds(a1, na - a1 - TH1)
        head = (pl.ds(na - TH1, TH1), pl.ds(0, S - NTAIL * TW1))
        tail = (pl.ds(na - TH1, TH1), pl.ds(S - NTAIL * TW1, NTAIL * TW1))
        copy(c_s.at[body_rows], buf_s.at[body_rows], sem.at[LC]).wait()
        copy(c_s.at[head], buf_s.at[head], sem.at[LC]).wait()
        queue_writes(0, INIT)
        copy(c_s.at[tail], buf_s.at[tail], sem.at[TL]).wait()

        def pair2(m, starts=()):
            g = m // G
            pair(m, jnp.where(g < neg, g % NR, NR + g - neg), m % G, starts)

        def body2(i, carry):
            for u in range(U2):
                k = i * U2 + u
                pair2(m1 + k, writes(k + INIT // PER, PER))
            return carry

        def body3(m, carry):
            pair2(m)
            return carry

        jax.lax.fori_loop(0, nb2, body2, 0)
        jax.lax.fori_loop(m1 + nb2 * U2, npair, body3, 0)
        queue_writes(rest0, nwt)
        copy(buf_s, o_hbm, sem.at[OUT]).wait()

    out = pl.pallas_call(
        kernel,
        in_specs=[pl.BlockSpec(memory_space=pl.ANY)] * 5,
        out_specs=pl.BlockSpec(memory_space=pl.ANY),
        out_shape=jax.ShapeDtypeStruct((na, S, C), c_fine.dtype),
        scratch_shapes=[
            pltpu.VMEM((npair, pw, C), bf16),
            pltpu.VMEM((NR + nlg, pg, C), bf16),
            pltpu.VMEM((C, C), bf16),
            pltpu.VMEM((C, C), bf16),
            pltpu.VMEM((C, C), bf16),
            pltpu.SemaphoreType.DMA((OUT + 1,)),
        ],
        compiler_params=pltpu.CompilerParams(
            vmem_limit_bytes=127 * 1024 * 1024,
            disable_bounds_checks=True,
        ),
    )(
        c_fine.reshape(npair, pw, C),
        c_fine.reshape(na, S, C),
        p_coarse.reshape(ng, pg, C),
        w_lat,
        w_out.reshape(C, C),
    )
    return out.reshape(B, H, W, C)
```

```python
import jax
import jax.numpy as jnp
import jax.experimental.pallas as pl
import jax.experimental.pallas.tpu as pltpu

G = 4
TW0 = 16
NE = 112
LEADG = 2
NR = 4
TH1, TW1 = 5, 8
THP, TWP = 4, 16
N1C, N1P = 13, 2
PRE1C, PRE1P = 140, 24
NSAT = 28
WSPLIT = 70
NTAIL = 16
S = 2048
TH, TW = 6, 16
INIT = 32
PER = 16
U1 = 2
U2 = 2
MT = 64
LAG = 2


def _weave(xs, ys):
    out, i, j = [], 0, 0
    while i < len(xs) or j < len(ys):
        if j < len(ys) and j * len(xs) <= i * len(ys):
            out.append(ys[j])
            j += 1
        else:
            out.append(xs[i])
            i += 1
    return out


def _div(i, n, limit):
    if isinstance(i, int) or n & (n - 1) == 0:
        return i // n
    magic = -(-(1 << 18) // n)
    assert limit * magic < 2**31 and all((x * magic) >> 18 == x // n for x in range(limit))
    return (i * magic) >> 18


def _aligned(x, k):
    return x if isinstance(x, int) else pl.multiple_of(x, k)


@jax.jit
def pallas_standalone__detection_seg_fpn_lateral__vision_kernel(
    c_fine: jax.Array,
    p_coarse: jax.Array,
    w_lat: jax.Array,
    w_out: jax.Array,
):
    B, H, W, C = c_fine.shape
    assert B == 1 and w_out.shape == (1, 1, C, C)
    assert p_coarse.shape == (1, H // 2, W // 2, C)
    f32, bf16 = jnp.float32, jnp.bfloat16
    npair, pw, pc = H // 2, 2 * W, W // 2
    pg = G * pc
    ng, neg = npair // G, NE // G
    nlg = ng - neg
    nig = neg - LEADG
    m1 = nig * G
    na = H * W // S
    assert npair % G == 0 and NE % G == 0 and G % U1 == 0 and NR > LEADG and (H * W) % S == 0
    px0, nw0 = G * TW0, pw // TW0
    n0c, n0p = nw0 // G, pc // px0
    assert pw % TW0 == 0 and nw0 % G == 0 and pc % px0 == 0
    nw1, nwp = pw // TW1, pg // TWP
    assert (npair - NE) % TH1 == 0 and pw % TW1 == 0 and nlg % THP == 0 and pg % TWP == 0
    n1c, n1p = (npair - NE) // TH1 * nw1, nlg // THP * nwp
    post1c, post1p = n1c - PRE1C - m1 * N1C, n1p - PRE1P - m1 * N1P
    assert NTAIL <= post1c and NTAIL < nw1 and post1p >= 0
    nwin = S // TW
    nwt = na // TH * nwin
    nb2 = min(npair - m1, (nwt - nwin - INIT) // PER) // U2
    rest0 = INIT + PER * nb2 * U2
    assert na % TH == 0 and S % TW == 0 and nwin % PER == 0 and INIT % PER == 0

    def pairs_needed(t):
        return -(-((t // nwin + 1) * TH * S) // pw)

    assert pairs_needed(INIT - 1) <= m1
    assert all(pairs_needed(INIT + PER * (k + 1) - 1) <= m1 + k for k in range(nb2 * U2))
    nt, nq = pw // MT, pc // MT
    assert pc % MT == 0 and W % MT == 0
    CS, PS, LC, LP, WT, TL, OUT = 0, NR, 2 * NR, 2 * NR + 1, 2 * NR + 2, 2 * NR + 3, 2 * NR + 4

    def kernel(c_pair, p_g, wl_hbm, wo_hbm, o_hbm, buf, pbuf, wl_v, wo_v, wf_v, sem):
        copy = pltpu.make_async_copy
        buf_s = buf.reshape(na, S, C)

        def early_c(g, k):
            at = (pl.ds(g * G, G), pl.ds(_aligned(k * TW0, TW0), TW0))
            return copy(c_pair.at[at], buf.at[at], sem.at[CS + g % NR])

        def early_p(g, k):
            px = pl.ds(_aligned(k * px0, px0), px0)
            return copy(p_g.at[g, px], pbuf.at[g % NR, px], sem.at[PS + g % NR])

        def wait_group(g):
            copy(p_g.at[g], pbuf.at[g % NR], sem.at[PS + g % NR]).wait()
            pairs = pl.ds(g * G, G)
            copy(c_pair.at[pairs], buf.at[pairs], sem.at[CS + g % NR]).wait()

        def late_c(i, s=LC):
            q = _div(i, nw1, n1c)
            at = (pl.ds(NE + q * TH1, TH1), pl.ds(_aligned((i - q * nw1) * TW1, TW1), TW1))
            return copy(c_pair.at[at], buf.at[at], sem.at[s])

        def late_p(i):
            q = _div(i, nwp, n1p)
            px = pl.ds(_aligned((i - q * nwp) * TWP, TWP), TWP)
            return copy(p_g.at[pl.ds(neg + q * THP, THP), px],
                        pbuf.at[pl.ds(NR + q * THP, THP), px], sem.at[LP])

        def start_write(a0, w0):
            win = (pl.ds(a0, TH), pl.ds(w0, TW))
            copy(buf_s.at[win], o_hbm.at[win], sem.at[OUT]).start()

        def writes(i, n):
            a0 = (i // (nwin // n)) * TH
            w0 = (i % (nwin // n)) * (n * TW)
            return [lambda k=k: start_write(a0, pl.multiple_of(w0 + k * TW, TW)) for k in range(n)]

        def queue_writes(lo, hi):
            def body(i, carry):
                for start in writes(i, 4):
                    start()
                return carry

            jax.lax.fori_loop(lo // 4, hi // 4, body, 0)

        def high(fn, *args):
            return lambda: fn(*args).start()

        def low(fn, *args):
            return lambda: fn(*args).start(priority=1)

        wl_cp = copy(wl_hbm, wl_v, sem.at[WT])
        wo_cp = copy(wo_hbm, wo_v, sem.at[WT])
        wl_cp.start()
        wo_cp.start()
        lows = _weave([low(late_c, i) for i in range(PRE1C)],
                      [low(late_p, i) for i in range(PRE1P)])
        highs = []
        for g in range(LEADG):
            highs += _weave([high(early_c, g, k) for k in range(nw0)],
                            [high(early_p, g, k) for k in range(G * n0p)])
        starts = lows[:NSAT] + _weave(highs, lows[NSAT:])
        for start in starts[:WSPLIT]:
            start()
        wl_cp.wait()
        wo_cp.wait()
        wf_v[...] = jnp.dot(wl_v[...], wo_v[...], preferred_element_type=f32).astype(bf16)
        for start in starts[WSPLIT:]:
            start()

        def pair(m, slot, j, starts=()):
            ups = []
            for i in range(nq):
                x = pbuf[slot, pl.ds(_aligned(j * pc + i * MT, MT), MT), :]
                q = jnp.dot(x, wo_v[...], preferred_element_type=f32)
                u = pltpu.bitcast(q.astype(bf16).astype(f32), jnp.uint32)
                ups.append(pltpu.bitcast(u | (u >> 16), bf16).astype(f32))
            up = jnp.concatenate(ups, axis=0)

            def mm(t):
                return jnp.dot(buf[m, pl.ds(t * MT, MT), :], wf_v[...],
                               preferred_element_type=f32)

            accs = [mm(t) for t in range(LAG)]
            for t in range(nt):
                if t + LAG < nt:
                    accs.append(mm(t + LAG))
                lo = (t * MT) % W
                buf[m, pl.ds(t * MT, MT), :] = (accs[t] + up[lo:lo + MT]).astype(bf16)
                for start in starts[t * len(starts) // nt:(t + 1) * len(starts) // nt]:
                    start()

        def group(g, carry):
            wait_group(g)

            def body(jj, c2):
                for u in range(U1):
                    j = jj * U1 + u
                    m = g * G + j
                    highs = _weave(
                        [high(early_c, g + LEADG, j * n0c + k) for k in range(n0c)],
                        [high(early_p, g + LEADG, j * n0p + k) for k in range(n0p)])
                    lows = _weave(
                        [low(late_c, PRE1C + m * N1C + k) for k in range(N1C)],
                        [low(late_p, PRE1P + m * N1P + k) for k in range(N1P)])
                    pair(m, g % NR, j, _weave(highs, lows))
                return c2

            jax.lax.fori_loop(0, G // U1, body, 0)
            return carry

        jax.lax.fori_loop(0, nig, group, 0)

        rest = _weave([(late_c, i) for i in range(n1c - post1c, n1c - NTAIL)],
                      [(late_p, i) for i in range(n1p - post1p, n1p)])
        for n, (fn, i) in enumerate(rest):
            fn(i).start(priority=(n + 1) % 2)
        for i in range(n1c - NTAIL, n1c):
            late_c(i, TL).start(priority=1)

        for g in range(nig, neg):
            wait_group(g)
        copy(p_g.at[pl.ds(neg, nlg)], pbuf.at[pl.ds(NR, nlg)], sem.at[LP]).wait()
        bulk = pl.ds(NE, npair - NE - TH1)
        head = (pl.ds(npair - TH1, TH1), pl.ds(0, pw - NTAIL * TW1))
        tail = (pl.ds(npair - TH1, TH1), pl.ds(pw - NTAIL * TW1, NTAIL * TW1))
        copy(c_pair.at[bulk], buf.at[bulk], sem.at[LC]).wait()
        copy(c_pair.at[head], buf.at[head], sem.at[LC]).wait()
        queue_writes(0, INIT)
        copy(c_pair.at[tail], buf.at[tail], sem.at[TL]).wait()

        def pair2(m, starts=()):
            g = m // G
            pair(m, jnp.where(g < neg, g % NR, NR + g - neg), m % G, starts)

        def body2(i, carry):
            for u in range(U2):
                k = i * U2 + u
                pair2(m1 + k, writes(k + INIT // PER, PER))
            return carry

        def body3(m, carry):
            pair2(m)
            return carry

        jax.lax.fori_loop(0, nb2, body2, 0)
        jax.lax.fori_loop(m1 + nb2 * U2, npair, body3, 0)
        queue_writes(rest0, nwt)
        copy(buf_s, o_hbm, sem.at[OUT]).wait()

    out = pl.pallas_call(
        kernel,
        in_specs=[pl.BlockSpec(memory_space=pl.ANY)] * 4,
        out_specs=pl.BlockSpec(memory_space=pl.ANY),
        out_shape=jax.ShapeDtypeStruct((na, S, C), c_fine.dtype),
        scratch_shapes=[
            pltpu.VMEM((npair, pw, C), bf16),
            pltpu.VMEM((NR + nlg, pg, C), bf16),
            pltpu.VMEM((C, C), bf16),
            pltpu.VMEM((C, C), bf16),
            pltpu.VMEM((C, C), bf16),
            pltpu.SemaphoreType.DMA((OUT + 1,)),
        ],
        compiler_params=pltpu.CompilerParams(
            vmem_limit_bytes=127 * 1024 * 1024,
            disable_bounds_checks=True,
        ),
    )(
        c_fine.reshape(npair, pw, C),
        p_coarse.reshape(ng, pg, C),
        w_lat,
        w_out.reshape(C, C),
    )
    return out.reshape(B, H, W, C)
```

```python
import jax
import jax.numpy as jnp
import jax.experimental.pallas as pl
import jax.experimental.pallas.tpu as pltpu

G = 4
TW0 = 16
NE = 112
LEADG = 2
NR = 4
TH1, TW1 = 4, 16
THP, TWP = 4, 16
N1C, N1P = 8, 2
PRE1C, PRE1P = 100, 24
NSAT = 28
WSPLIT = 70
NTAIL = 10
S = 2048
TH, TW = 6, 16
INIT = 32
PER = 16
U1 = 2
U2 = 2
MT = 64
LAG = 2


def _weave(xs, ys):
    out, i, j = [], 0, 0
    while i < len(xs) or j < len(ys):
        if j < len(ys) and j * len(xs) <= i * len(ys):
            out.append(ys[j])
            j += 1
        else:
            out.append(xs[i])
            i += 1
    return out


def _div(i, n, limit):
    if isinstance(i, int) or n & (n - 1) == 0:
        return i // n
    magic = -(-(1 << 18) // n)
    assert limit * magic < 2**31 and all((x * magic) >> 18 == x // n for x in range(limit))
    return (i * magic) >> 18


def _aligned(x, k):
    return x if isinstance(x, int) else pl.multiple_of(x, k)


@jax.jit
def pallas_standalone__detection_seg_fpn_lateral__vision_kernel(
    c_fine: jax.Array,
    p_coarse: jax.Array,
    w_lat: jax.Array,
    w_out: jax.Array,
):
    B, H, W, C = c_fine.shape
    assert B == 1 and w_out.shape == (1, 1, C, C)
    assert p_coarse.shape == (1, H // 2, W // 2, C)
    f32, bf16 = jnp.float32, jnp.bfloat16
    npair, pw, pc = H // 2, 2 * W, W // 2
    pg = G * pc
    ng, neg = npair // G, NE // G
    nlg = ng - neg
    nig = neg - LEADG
    m1 = nig * G
    na = H * W // S
    assert npair % G == 0 and NE % G == 0 and G % U1 == 0 and NR > LEADG and (H * W) % S == 0
    px0, nw0 = G * TW0, pw // TW0
    n0c, n0p = nw0 // G, pc // px0
    assert pw % TW0 == 0 and nw0 % G == 0 and pc % px0 == 0
    nw1, nwp = pw // TW1, pg // TWP
    assert (npair - NE) % TH1 == 0 and pw % TW1 == 0 and nlg % THP == 0 and pg % TWP == 0
    n1c, n1p = (npair - NE) // TH1 * nw1, nlg // THP * nwp
    post1c, post1p = n1c - PRE1C - m1 * N1C, n1p - PRE1P - m1 * N1P
    assert NTAIL <= post1c and NTAIL < nw1 and post1p >= 0
    nwin = S // TW
    nwt = na // TH * nwin
    nb2 = min(npair - m1, (nwt - nwin - INIT) // PER) // U2
    rest0 = INIT + PER * nb2 * U2
    assert na % TH == 0 and S % TW == 0 and nwin % PER == 0 and INIT % PER == 0

    def pairs_needed(t):
        return -(-((t // nwin + 1) * TH * S) // pw)

    assert pairs_needed(INIT - 1) <= m1
    assert all(pairs_needed(INIT + PER * (k + 1) - 1) <= m1 + k for k in range(nb2 * U2))
    nt, nq = pw // MT, pc // MT
    assert pc % MT == 0 and W % MT == 0
    CS, PS, LC, LP, WT, TL, OUT = 0, NR, 2 * NR, 2 * NR + 1, 2 * NR + 2, 2 * NR + 3, 2 * NR + 4

    def kernel(c_pair, p_g, wl_hbm, wo_hbm, o_hbm, buf, pbuf, wl_v, wo_v, wf_v, sem):
        copy = pltpu.make_async_copy
        buf_s = buf.reshape(na, S, C)

        def early_c(g, k):
            at = (pl.ds(g * G, G), pl.ds(_aligned(k * TW0, TW0), TW0))
            return copy(c_pair.at[at], buf.at[at], sem.at[CS + g % NR])

        def early_p(g, k):
            px = pl.ds(_aligned(k * px0, px0), px0)
            return copy(p_g.at[g, px], pbuf.at[g % NR, px], sem.at[PS + g % NR])

        def wait_group(g):
            copy(p_g.at[g], pbuf.at[g % NR], sem.at[PS + g % NR]).wait()
            pairs = pl.ds(g * G, G)
            copy(c_pair.at[pairs], buf.at[pairs], sem.at[CS + g % NR]).wait()

        def late_c(i, s=LC):
            q = _div(i, nw1, n1c)
            at = (pl.ds(NE + q * TH1, TH1), pl.ds(_aligned((i - q * nw1) * TW1, TW1), TW1))
            return copy(c_pair.at[at], buf.at[at], sem.at[s])

        def late_p(i):
            q = _div(i, nwp, n1p)
            px = pl.ds(_aligned((i - q * nwp) * TWP, TWP), TWP)
            return copy(p_g.at[pl.ds(neg + q * THP, THP), px],
                        pbuf.at[pl.ds(NR + q * THP, THP), px], sem.at[LP])

        def start_write(a0, w0):
            win = (pl.ds(a0, TH), pl.ds(w0, TW))
            copy(buf_s.at[win], o_hbm.at[win], sem.at[OUT]).start()

        def writes(i, n):
            a0 = (i // (nwin // n)) * TH
            w0 = (i % (nwin // n)) * (n * TW)
            return [lambda k=k: start_write(a0, pl.multiple_of(w0 + k * TW, TW)) for k in range(n)]

        def queue_writes(lo, hi):
            def body(i, carry):
                for start in writes(i, 4):
                    start()
                return carry

            jax.lax.fori_loop(lo // 4, hi // 4, body, 0)

        def high(fn, *args):
            return lambda: fn(*args).start()

        def low(fn, *args):
            return lambda: fn(*args).start(priority=1)

        wl_cp = copy(wl_hbm, wl_v, sem.at[WT])
        wo_cp = copy(wo_hbm, wo_v, sem.at[WT])
        wl_cp.start()
        wo_cp.start()
        lows = _weave([low(late_c, i) for i in range(PRE1C)],
                      [low(late_p, i) for i in range(PRE1P)])
        highs = []
        for g in range(LEADG):
            highs += _weave([high(early_c, g, k) for k in range(nw0)],
                            [high(early_p, g, k) for k in range(G * n0p)])
        starts = lows[:NSAT] + _weave(highs, lows[NSAT:])
        for start in starts[:WSPLIT]:
            start()
        wl_cp.wait()
        wo_cp.wait()
        wf_v[...] = jnp.dot(wl_v[...], wo_v[...], preferred_element_type=f32).astype(bf16)
        for start in starts[WSPLIT:]:
            start()

        def pair(m, slot, j, starts=()):
            ups = []
            for i in range(nq):
                x = pbuf[slot, pl.ds(_aligned(j * pc + i * MT, MT), MT), :]
                q = jnp.dot(x, wo_v[...], preferred_element_type=f32)
                u = pltpu.bitcast(q.astype(bf16).astype(f32), jnp.uint32)
                ups.append(pltpu.bitcast(u | (u >> 16), bf16).astype(f32))
            up = jnp.concatenate(ups, axis=0)

            def mm(t):
                return jnp.dot(buf[m, pl.ds(t * MT, MT), :], wf_v[...],
                               preferred_element_type=f32)

            accs = [mm(t) for t in range(LAG)]
            for t in range(nt):
                if t + LAG < nt:
                    accs.append(mm(t + LAG))
                lo = (t * MT) % W
                buf[m, pl.ds(t * MT, MT), :] = (accs[t] + up[lo:lo + MT]).astype(bf16)
                for start in starts[t * len(starts) // nt:(t + 1) * len(starts) // nt]:
                    start()

        def group(g, carry):
            wait_group(g)

            def body(jj, c2):
                for u in range(U1):
                    j = jj * U1 + u
                    m = g * G + j
                    highs = _weave(
                        [high(early_c, g + LEADG, j * n0c + k) for k in range(n0c)],
                        [high(early_p, g + LEADG, j * n0p + k) for k in range(n0p)])
                    lows = _weave(
                        [low(late_c, PRE1C + m * N1C + k) for k in range(N1C)],
                        [low(late_p, PRE1P + m * N1P + k) for k in range(N1P)])
                    pair(m, g % NR, j, _weave(highs, lows))
                return c2

            jax.lax.fori_loop(0, G // U1, body, 0)
            return carry

        jax.lax.fori_loop(0, nig, group, 0)

        rest = _weave([(late_c, i) for i in range(n1c - post1c, n1c - NTAIL)],
                      [(late_p, i) for i in range(n1p - post1p, n1p)])
        for n, (fn, i) in enumerate(rest):
            fn(i).start(priority=(n + 1) % 2)
        for i in range(n1c - NTAIL, n1c):
            late_c(i, TL).start(priority=1)

        for g in range(nig, neg):
            wait_group(g)
        copy(p_g.at[pl.ds(neg, nlg)], pbuf.at[pl.ds(NR, nlg)], sem.at[LP]).wait()
        bulk = pl.ds(NE, npair - NE - TH1)
        head = (pl.ds(npair - TH1, TH1), pl.ds(0, pw - NTAIL * TW1))
        tail = (pl.ds(npair - TH1, TH1), pl.ds(pw - NTAIL * TW1, NTAIL * TW1))
        copy(c_pair.at[bulk], buf.at[bulk], sem.at[LC]).wait()
        copy(c_pair.at[head], buf.at[head], sem.at[LC]).wait()
        queue_writes(0, INIT)
        copy(c_pair.at[tail], buf.at[tail], sem.at[TL]).wait()

        def pair2(m, starts=()):
            g = m // G
            pair(m, jnp.where(g < neg, g % NR, NR + g - neg), m % G, starts)

        def body2(i, carry):
            for u in range(U2):
                k = i * U2 + u
                pair2(m1 + k, writes(k + INIT // PER, PER))
            return carry

        def body3(m, carry):
            pair2(m)
            return carry

        jax.lax.fori_loop(0, nb2, body2, 0)
        jax.lax.fori_loop(m1 + nb2 * U2, npair, body3, 0)
        queue_writes(rest0, nwt)
        copy(buf_s, o_hbm, sem.at[OUT]).wait()

    out = pl.pallas_call(
        kernel,
        in_specs=[pl.BlockSpec(memory_space=pl.ANY)] * 4,
        out_specs=pl.BlockSpec(memory_space=pl.ANY),
        out_shape=jax.ShapeDtypeStruct((na, S, C), c_fine.dtype),
        scratch_shapes=[
            pltpu.VMEM((npair, pw, C), bf16),
            pltpu.VMEM((NR + nlg, pg, C), bf16),
            pltpu.VMEM((C, C), bf16),
            pltpu.VMEM((C, C), bf16),
            pltpu.VMEM((C, C), bf16),
            pltpu.SemaphoreType.DMA((OUT + 1,)),
        ],
        compiler_params=pltpu.CompilerParams(
            vmem_limit_bytes=127 * 1024 * 1024,
            disable_bounds_checks=True,
        ),
    )(
        c_fine.reshape(npair, pw, C),
        p_coarse.reshape(ng, pg, C),
        w_lat,
        w_out.reshape(C, C),
    )
    return out.reshape(B, H, W, C)
```

```python
import jax
import jax.numpy as jnp
import jax.experimental.pallas as pl
import jax.experimental.pallas.tpu as pltpu

G = 4
TW0 = 16
NE = 112
LEADG = 2
NR = 4
TH1, TW1 = 4, 16
THP, TWP = 4, 16
N1C, N1P = 8, 2
PRE1C, PRE1P = 100, 24
NSAT = 28
WSPLIT = 70
NTAIL = 10
S = 2048
TH, TW = 6, 16
INIT = 64
PER = 16
X1 = 1
U2 = 4
MT = 64
LAG = 2


def _weave(xs, ys):
    out, i, j = [], 0, 0
    while i < len(xs) or j < len(ys):
        if j < len(ys) and j * len(xs) <= i * len(ys):
            out.append(ys[j])
            j += 1
        else:
            out.append(xs[i])
            i += 1
    return out


def _div(i, n, limit):
    if isinstance(i, int) or n & (n - 1) == 0:
        return i // n
    magic = -(-(1 << 18) // n)
    assert limit * magic < 2**31 and all((x * magic) >> 18 == x // n for x in range(limit))
    return (i * magic) >> 18


def _aligned(x, k):
    return x if isinstance(x, int) else pl.multiple_of(x, k)


@jax.jit
def pallas_standalone__detection_seg_fpn_lateral__vision_kernel(
    c_fine: jax.Array,
    p_coarse: jax.Array,
    w_lat: jax.Array,
    w_out: jax.Array,
):
    B, H, W, C = c_fine.shape
    assert B == 1 and w_out.shape == (1, 1, C, C)
    assert p_coarse.shape == (1, H // 2, W // 2, C)
    f32, bf16 = jnp.float32, jnp.bfloat16
    npair, pw, pc = H // 2, 2 * W, W // 2
    pg = G * pc
    ng, neg = npair // G, NE // G
    nlg = ng - neg
    nig = neg - LEADG
    ni = nig * G
    m1 = ni + X1
    na = H * W // S
    assert npair % G == 0 and NE % G == 0 and NR > LEADG and m1 <= NE and (H * W) % S == 0
    px0, nw0 = G * TW0, pw // TW0
    n0c, n0p = nw0 // G, pc // px0
    assert pw % TW0 == 0 and nw0 % G == 0 and pc % px0 == 0
    nw1, nwp = pw // TW1, pg // TWP
    assert (npair - NE) % TH1 == 0 and pw % TW1 == 0 and nlg % THP == 0 and pg % TWP == 0
    n1c, n1p = (npair - NE) // TH1 * nw1, nlg // THP * nwp
    post1c, post1p = n1c - PRE1C - ni * N1C, n1p - PRE1P - ni * N1P
    assert NTAIL <= post1c and NTAIL < nw1 and post1p >= 0
    nwin = S // TW
    nwt = na // TH * nwin
    nb2 = min(npair - m1, (nwt - nwin - INIT) // PER) // U2
    rest0 = INIT + PER * nb2 * U2
    assert na % TH == 0 and S % TW == 0 and nwin % PER == 0 and INIT % PER == 0

    def pairs_needed(t):
        return -(-((t // nwin + 1) * TH * S) // pw)

    assert pairs_needed(INIT - 1) <= m1
    assert all(pairs_needed(INIT + PER * (k + 1) - 1) <= m1 + k for k in range(nb2 * U2))
    nt, nq = pw // MT, pc // MT
    assert pc % MT == 0 and W % MT == 0
    CS, PS, LC, LP, WT, TL, OUT = 0, NR, 2 * NR, 2 * NR + 1, 2 * NR + 2, 2 * NR + 3, 2 * NR + 4

    def kernel(c_pair, p_g, wl_hbm, wo_hbm, o_hbm, buf, pbuf, wl_v, wo_v, wf_v, sem):
        copy = pltpu.make_async_copy
        buf_s = buf.reshape(na, S, C)

        def early_c(g, k):
            at = (pl.ds(g * G, G), pl.ds(_aligned(k * TW0, TW0), TW0))
            return copy(c_pair.at[at], buf.at[at], sem.at[CS + g % NR])

        def early_p(g, k):
            px = pl.ds(_aligned(k * px0, px0), px0)
            return copy(p_g.at[g, px], pbuf.at[g % NR, px], sem.at[PS + g % NR])

        def wait_group(g):
            copy(p_g.at[g], pbuf.at[g % NR], sem.at[PS + g % NR]).wait()
            pairs = pl.ds(g * G, G)
            copy(c_pair.at[pairs], buf.at[pairs], sem.at[CS + g % NR]).wait()

        def late_c(i, s=LC):
            q = _div(i, nw1, n1c)
            at = (pl.ds(NE + q * TH1, TH1), pl.ds(_aligned((i - q * nw1) * TW1, TW1), TW1))
            return copy(c_pair.at[at], buf.at[at], sem.at[s])

        def late_p(i):
            q = _div(i, nwp, n1p)
            px = pl.ds(_aligned((i - q * nwp) * TWP, TWP), TWP)
            return copy(p_g.at[pl.ds(neg + q * THP, THP), px],
                        pbuf.at[pl.ds(NR + q * THP, THP), px], sem.at[LP])

        def start_write(a0, w0):
            win = (pl.ds(a0, TH), pl.ds(w0, TW))
            copy(buf_s.at[win], o_hbm.at[win], sem.at[OUT]).start()

        def writes(i, n):
            a0 = (i // (nwin // n)) * TH
            w0 = (i % (nwin // n)) * (n * TW)
            return [lambda k=k: start_write(a0, pl.multiple_of(w0 + k * TW, TW)) for k in range(n)]

        def queue_writes(lo, hi):
            def body(i, carry):
                for start in writes(i, 4):
                    start()
                return carry

            jax.lax.fori_loop(lo // 4, hi // 4, body, 0)

        def high(fn, *args):
            return lambda: fn(*args).start()

        def low(fn, *args):
            return lambda: fn(*args).start(priority=1)

        wl_cp = copy(wl_hbm, wl_v, sem.at[WT])
        wo_cp = copy(wo_hbm, wo_v, sem.at[WT])
        wl_cp.start()
        wo_cp.start()
        lows = _weave([low(late_c, i) for i in range(PRE1C)],
                      [low(late_p, i) for i in range(PRE1P)])
        highs = []
        for g in range(LEADG):
            highs += _weave([high(early_c, g, k) for k in range(nw0)],
                            [high(early_p, g, k) for k in range(G * n0p)])
        starts = lows[:NSAT] + _weave(highs, lows[NSAT:])
        for start in starts[:WSPLIT]:
            start()
        wl_cp.wait()
        wo_cp.wait()
        wf_v[...] = jnp.dot(wl_v[...], wo_v[...], preferred_element_type=f32).astype(bf16)
        for start in starts[WSPLIT:]:
            start()

        def pair(m, slot, j, starts=()):
            ups = []
            for i in range(nq):
                x = pbuf[slot, pl.ds(_aligned(j * pc + i * MT, MT), MT), :]
                q = jnp.dot(x, wo_v[...], preferred_element_type=f32)
                u = pltpu.bitcast(q.astype(bf16).astype(f32), jnp.uint32)
                ups.append(pltpu.bitcast(u | (u >> 16), bf16).astype(f32))
            up = jnp.concatenate(ups, axis=0)

            def mm(t):
                return jnp.dot(buf[m, pl.ds(t * MT, MT), :], wf_v[...],
                               preferred_element_type=f32)

            accs = [mm(t) for t in range(LAG)]
            for t in range(nt):
                if t + LAG < nt:
                    accs.append(mm(t + LAG))
                lo = (t * MT) % W
                buf[m, pl.ds(t * MT, MT), :] = (accs[t] + up[lo:lo + MT]).astype(bf16)
                for start in starts[t * len(starts) // nt:(t + 1) * len(starts) // nt]:
                    start()

        def group(g, carry):
            wait_group(g)
            for j in range(G):
                m = g * G + j
                highs = _weave(
                    [high(early_c, g + LEADG, j * n0c + k) for k in range(n0c)],
                    [high(early_p, g + LEADG, j * n0p + k) for k in range(n0p)])
                lows = _weave(
                    [low(late_c, PRE1C + m * N1C + k) for k in range(N1C)],
                    [low(late_p, PRE1P + m * N1P + k) for k in range(N1P)])
                pair(m, g % NR, j, _weave(highs, lows))
            return carry

        jax.lax.fori_loop(0, nig, group, 0)

        rest = _weave([(late_c, i) for i in range(n1c - post1c, n1c - NTAIL)],
                      [(late_p, i) for i in range(n1p - post1p, n1p)])
        for n, (fn, i) in enumerate(rest):
            fn(i).start(priority=(n + 1) % 2)
        for i in range(n1c - NTAIL, n1c):
            late_c(i, TL).start(priority=1)

        def any_pair(m, starts=()):
            g = m // G
            pair(m, jnp.where(g < neg, g % NR, NR + g - neg), m % G, starts)

        def plain(m, carry):
            any_pair(m)
            return carry

        for g in range(nig, neg):
            wait_group(g)
        jax.lax.fori_loop(ni, m1, plain, 0)

        copy(p_g.at[pl.ds(neg, nlg)], pbuf.at[pl.ds(NR, nlg)], sem.at[LP]).wait()
        bulk = pl.ds(NE, npair - NE - TH1)
        head = (pl.ds(npair - TH1, TH1), pl.ds(0, pw - NTAIL * TW1))
        tail = (pl.ds(npair - TH1, TH1), pl.ds(pw - NTAIL * TW1, NTAIL * TW1))
        copy(c_pair.at[bulk], buf.at[bulk], sem.at[LC]).wait()
        copy(c_pair.at[head], buf.at[head], sem.at[LC]).wait()
        queue_writes(0, INIT)
        copy(c_pair.at[tail], buf.at[tail], sem.at[TL]).wait()

        def body2(i, carry):
            for u in range(U2):
                k = i * U2 + u
                any_pair(m1 + k, writes(k + INIT // PER, PER))
            return carry

        jax.lax.fori_loop(0, nb2, body2, 0)
        jax.lax.fori_loop(m1 + nb2 * U2, npair, plain, 0)
        queue_writes(rest0, nwt)
        copy(buf_s, o_hbm, sem.at[OUT]).wait()

    out = pl.pallas_call(
        kernel,
        in_specs=[pl.BlockSpec(memory_space=pl.ANY)] * 4,
        out_specs=pl.BlockSpec(memory_space=pl.ANY),
        out_shape=jax.ShapeDtypeStruct((na, S, C), c_fine.dtype),
        scratch_shapes=[
            pltpu.VMEM((npair, pw, C), bf16),
            pltpu.VMEM((NR + nlg, pg, C), bf16),
            pltpu.VMEM((C, C), bf16),
            pltpu.VMEM((C, C), bf16),
            pltpu.VMEM((C, C), bf16),
            pltpu.SemaphoreType.DMA((OUT + 1,)),
        ],
        compiler_params=pltpu.CompilerParams(vmem_limit_bytes=127 * 1024 * 1024),
    )(
        c_fine.reshape(npair, pw, C),
        p_coarse.reshape(ng, pg, C),
        w_lat,
        w_out.reshape(C, C),
    )
    return out.reshape(B, H, W, C)
```

```python
import jax
import jax.numpy as jnp
import jax.experimental.pallas as pl
import jax.experimental.pallas.tpu as pltpu

G = 4
TW0 = 16
NE = 112
LEADG = 2
NR = 4
TH1, TW1 = 4, 16
THP, TWP = 4, 16
N1C, N1P = 8, 2
PRE1C, PRE1P = 96, 24
NSAT = 28
WSPLIT = 70
NTAIL = 10
S = 2048
TH, TW = 6, 16
INIT = 64
PER = 16
X1 = 1
U2 = 4
MT = 64
LAG = 2


def _weave(xs, ys):
    out, i, j = [], 0, 0
    while i < len(xs) or j < len(ys):
        if j < len(ys) and j * len(xs) <= i * len(ys):
            out.append(ys[j])
            j += 1
        else:
            out.append(xs[i])
            i += 1
    return out


def _aligned(x, k):
    return x if isinstance(x, int) else pl.multiple_of(x, k)


@jax.jit
def pallas_standalone__detection_seg_fpn_lateral__vision_kernel(
    c_fine: jax.Array,
    p_coarse: jax.Array,
    w_lat: jax.Array,
    w_out: jax.Array,
):
    B, H, W, C = c_fine.shape
    assert B == 1 and w_out.shape == (1, 1, C, C)
    assert p_coarse.shape == (1, H // 2, W // 2, C)
    f32, bf16 = jnp.float32, jnp.bfloat16
    npair, pw, pc = H // 2, 2 * W, W // 2
    pg = G * pc
    ng, neg = npair // G, NE // G
    nlg = ng - neg
    nig = neg - LEADG
    ni = nig * G
    m1 = ni + X1
    na = H * W // S
    assert npair % G == 0 and NE % G == 0 and NR > LEADG and m1 <= NE and (H * W) % S == 0
    px0, nw0 = G * TW0, pw // TW0
    n0c, n0p = nw0 // G, pc // px0
    assert pw % TW0 == 0 and nw0 % G == 0 and pc % px0 == 0
    nw1, nwp = pw // TW1, pg // TWP
    assert (npair - NE) % TH1 == 0 and pw % TW1 == 0 and nlg % THP == 0 and pg % TWP == 0
    n1c, n1p = (npair - NE) // TH1 * nw1, nlg // THP * nwp
    post1c, post1p = n1c - PRE1C - ni * N1C, n1p - PRE1P - ni * N1P
    assert NTAIL <= post1c and NTAIL < nw1 and post1p >= 0
    assert PRE1C % N1C == 0 and nw1 % N1C == 0 and PRE1P % N1P == 0 and nwp % N1P == 0
    nwin = S // TW
    nwt = na // TH * nwin
    nb2 = min(npair - m1, (nwt - nwin - INIT) // PER) // U2
    rest0 = INIT + PER * nb2 * U2
    assert na % TH == 0 and S % TW == 0 and nwin % PER == 0 and INIT % PER == 0

    def pairs_needed(t):
        return -(-((t // nwin + 1) * TH * S) // pw)

    assert pairs_needed(INIT - 1) <= m1
    assert all(pairs_needed(INIT + PER * (k + 1) - 1) <= m1 + k for k in range(nb2 * U2))
    nt, nq = pw // MT, pc // MT
    assert pc % MT == 0 and W % MT == 0
    CS, PS, LC, LP, WT, TL, OUT = 0, NR, 2 * NR, 2 * NR + 1, 2 * NR + 2, 2 * NR + 3, 2 * NR + 4

    def kernel(c_pair, p_g, wl_hbm, wo_hbm, o_hbm, buf, pbuf, wl_v, wo_v, wf_v, sem):
        copy = pltpu.make_async_copy
        buf_s = buf.reshape(na, S, C)

        def early_c(g, k):
            at = (pl.ds(g * G, G), pl.ds(_aligned(k * TW0, TW0), TW0))
            return copy(c_pair.at[at], buf.at[at], sem.at[CS + g % NR])

        def early_p(g, k):
            px = pl.ds(_aligned(k * px0, px0), px0)
            return copy(p_g.at[g, px], pbuf.at[g % NR, px], sem.at[PS + g % NR])

        def wait_group(g):
            copy(p_g.at[g], pbuf.at[g % NR], sem.at[PS + g % NR]).wait()
            pairs = pl.ds(g * G, G)
            copy(c_pair.at[pairs], buf.at[pairs], sem.at[CS + g % NR]).wait()

        def late_c(q, k, s=LC):
            at = (pl.ds(NE + q * TH1, TH1), pl.ds(_aligned(k * TW1, TW1), TW1))
            return copy(c_pair.at[at], buf.at[at], sem.at[s])

        def late_p(q, k):
            px = pl.ds(_aligned(k * TWP, TWP), TWP)
            return copy(p_g.at[pl.ds(neg + q * THP, THP), px],
                        pbuf.at[pl.ds(NR + q * THP, THP), px], sem.at[LP])

        def start_write(a0, w0):
            win = (pl.ds(a0, TH), pl.ds(w0, TW))
            copy(buf_s.at[win], o_hbm.at[win], sem.at[OUT]).start()

        def writes(i, n):
            a0 = (i // (nwin // n)) * TH
            w0 = (i % (nwin // n)) * (n * TW)
            return [lambda k=k: start_write(a0, pl.multiple_of(w0 + k * TW, TW)) for k in range(n)]

        def queue_writes(lo, hi):
            assert lo % 4 == 0 and hi % 4 == 0

            def body(i, carry):
                for start in writes(i, 4):
                    start()
                return carry

            jax.lax.fori_loop(lo // 4, hi // 4, body, 0)

        def high(fn, *args):
            return lambda: fn(*args).start()

        def low(fn, *args):
            return lambda: fn(*args).start(priority=1)

        wl_cp = copy(wl_hbm, wl_v, sem.at[WT])
        wo_cp = copy(wo_hbm, wo_v, sem.at[WT])
        wl_cp.start()
        wo_cp.start()
        lows = _weave([low(late_c, *divmod(i, nw1)) for i in range(PRE1C)],
                      [low(late_p, *divmod(i, nwp)) for i in range(PRE1P)])
        highs = []
        for g in range(LEADG):
            highs += _weave([high(early_c, g, k) for k in range(nw0)],
                            [high(early_p, g, k) for k in range(G * n0p)])
        starts = lows[:NSAT] + _weave(highs, lows[NSAT:])
        for start in starts[:WSPLIT]:
            start()
        wl_cp.wait()
        wo_cp.wait()
        wf_v[...] = jnp.dot(wl_v[...], wo_v[...], preferred_element_type=f32).astype(bf16)
        for start in starts[WSPLIT:]:
            start()

        def pair(m, slot, j, starts=()):
            ups = []
            for i in range(nq):
                x = pbuf[slot, pl.ds(_aligned(j * pc + i * MT, MT), MT), :]
                q = jnp.dot(x, wo_v[...], preferred_element_type=f32)
                u = pltpu.bitcast(q.astype(bf16).astype(f32), jnp.uint32)
                ups.append(pltpu.bitcast(u | (u >> 16), bf16).astype(f32))
            up = jnp.concatenate(ups, axis=0)

            def mm(t):
                return jnp.dot(buf[m, pl.ds(t * MT, MT), :], wf_v[...],
                               preferred_element_type=f32)

            accs = [mm(t) for t in range(LAG)]
            for t in range(nt):
                if t + LAG < nt:
                    accs.append(mm(t + LAG))
                lo = (t * MT) % W
                buf[m, pl.ds(t * MT, MT), :] = (accs[t] + up[lo:lo + MT]).astype(bf16)
                for start in starts[t * len(starts) // nt:(t + 1) * len(starts) // nt]:
                    start()

        def group(g, carry):
            wait_group(g)
            for j in range(G):
                m = g * G + j
                highs = _weave(
                    [high(early_c, g + LEADG, j * n0c + k) for k in range(n0c)],
                    [high(early_p, g + LEADG, j * n0p + k) for k in range(n0p)])
                ic, ip = PRE1C // N1C + m, PRE1P // N1P + m
                qc, kc = ic // (nw1 // N1C), ic % (nw1 // N1C) * N1C
                qp, kp = ip // (nwp // N1P), ip % (nwp // N1P) * N1P
                lows = _weave([low(late_c, qc, kc + k) for k in range(N1C)],
                              [low(late_p, qp, kp + k) for k in range(N1P)])
                pair(m, g % NR, j, _weave(highs, lows))
            return carry

        jax.lax.fori_loop(0, nig, group, 0)

        rest = _weave([(late_c, divmod(i, nw1)) for i in range(n1c - post1c, n1c - NTAIL)],
                      [(late_p, divmod(i, nwp)) for i in range(n1p - post1p, n1p)])
        for n, (fn, at) in enumerate(rest):
            fn(*at).start(priority=(n + 1) % 2)
        for i in range(n1c - NTAIL, n1c):
            late_c(*divmod(i, nw1), TL).start(priority=1)

        def any_pair(m, starts=()):
            g = m // G
            pair(m, jnp.where(g < neg, g % NR, NR + g - neg), m % G, starts)

        def plain(m, carry):
            any_pair(m)
            return carry

        for g in range(nig, neg):
            wait_group(g)
        jax.lax.fori_loop(ni, m1, plain, 0)

        copy(p_g.at[pl.ds(neg, nlg)], pbuf.at[pl.ds(NR, nlg)], sem.at[LP]).wait()
        bulk = pl.ds(NE, npair - NE - TH1)
        head = (pl.ds(npair - TH1, TH1), pl.ds(0, pw - NTAIL * TW1))
        tail = (pl.ds(npair - TH1, TH1), pl.ds(pw - NTAIL * TW1, NTAIL * TW1))
        copy(c_pair.at[bulk], buf.at[bulk], sem.at[LC]).wait()
        copy(c_pair.at[head], buf.at[head], sem.at[LC]).wait()
        queue_writes(0, INIT)
        copy(c_pair.at[tail], buf.at[tail], sem.at[TL]).wait()

        def body2(i, carry):
            for u in range(U2):
                k = i * U2 + u
                any_pair(m1 + k, writes(k + INIT // PER, PER))
            return carry

        jax.lax.fori_loop(0, nb2, body2, 0)
        jax.lax.fori_loop(m1 + nb2 * U2, npair, plain, 0)
        queue_writes(rest0, nwt)
        copy(buf_s, o_hbm, sem.at[OUT]).wait()

    out = pl.pallas_call(
        kernel,
        in_specs=[pl.BlockSpec(memory_space=pl.ANY)] * 4,
        out_specs=pl.BlockSpec(memory_space=pl.ANY),
        out_shape=jax.ShapeDtypeStruct((na, S, C), c_fine.dtype),
        scratch_shapes=[
            pltpu.VMEM((npair, pw, C), bf16),
            pltpu.VMEM((NR + nlg, pg, C), bf16),
            pltpu.VMEM((C, C), bf16),
            pltpu.VMEM((C, C), bf16),
            pltpu.VMEM((C, C), bf16),
            pltpu.SemaphoreType.DMA((OUT + 1,)),
        ],
        compiler_params=pltpu.CompilerParams(vmem_limit_bytes=127 * 1024 * 1024),
    )(
        c_fine.reshape(npair, pw, C),
        p_coarse.reshape(ng, pg, C),
        w_lat,
        w_out.reshape(C, C),
    )
    return out.reshape(B, H, W, C)
```
